```python
import os as _os
_os.environ.setdefault("JAX_PLATFORMS", "cpu")
import jax
import jax.numpy as jnp

def _softmax(x, axis=-1):
    return jax.nn.softmax(x, axis=axis)
def _gelu(x):
    return jax.nn.gelu(x, approximate=True)
def _silu(x):
    return jax.nn.silu(x)
def _sigmoid(x):
    return jax.nn.sigmoid(x)
def _layernorm(x, axis=-1, eps=1e-5):
    m = jnp.mean(x, axis=axis, keepdims=True)
    v = jnp.var(x, axis=axis, keepdims=True)
    return (x - m) / jnp.sqrt(v + eps)
def _scatter_add(tgt, idx, src, axis=0):
    return tgt.at[idx].add(src)
def _segment_sum(src, seg, n):
    return jax.ops.segment_sum(src, seg, n)
class _Rng:
    def __init__(self, key):
        self._k = key
    def _next(self):
        self._k, sub = jax.random.split(self._k)
        return sub
    def normal(self, shape):
        return jax.random.normal(self._next(), shape, dtype=jnp.bfloat16)
    def randint(self, lo, hi, shape):
        return jax.random.randint(self._next(), shape, lo, hi, dtype=jnp.int32)
    def uniform(self, shape, lo=0.0, hi=1.0):
        return jax.random.uniform(self._next(), shape, jnp.bfloat16, lo, hi)
    def permutation(self, n):
        return jax.random.permutation(self._next(), n)


kernel_name = 'sequential_preLN__sliding_block__swiglu_ffn__prompt'

def setup_inputs():
    _rng = _Rng(jax.random.key(int.from_bytes(__import__("os").urandom(4), "little")))
    _w = (lambda a: (lambda t: t.astype(jnp.bfloat16) if jnp.issubdtype(t.dtype, jnp.floating) else t)(jnp.asarray(a)))
    def _A_setup():
        B, S, D = 1, 2048, 512
        return {
            "x": _w((lambda *s: _rng.normal(s) * 0.05)(B, S, D)),
            "wqkv": _w((lambda *s: _rng.normal(s) * 0.05)(D, 3 * D)),
            "wo": _w((lambda *s: _rng.normal(s) * 0.05)(D, D)),
        }
    _A_in = _A_setup()

    def _B_setup():
        B, S, D, F = 1, 2048, 512, 1792
        return {
            "x": _w((lambda *s: _rng.normal(s) * 0.05)(B, S, D)),
            "w_gate": _w((lambda *s: _rng.normal(s) * 0.05)(D, F)),
            "w_up": _w((lambda *s: _rng.normal(s) * 0.05)(D, F)),
            "w_down": _w((lambda *s: _rng.normal(s) * 0.05)(F, D)),
        }
    _B_in = _B_setup()

    return {
        "A_x": _A_in["x"],
        "A_wqkv": _A_in["wqkv"],
        "A_wo": _A_in["wo"],
        "B_x": _B_in["x"],
        "B_w_gate": _B_in["w_gate"],
        "B_w_up": _B_in["w_up"],
        "B_w_down": _B_in["w_down"],
    }

def reference(A_x, A_wqkv, A_wo, B_x, B_w_gate, B_w_up, B_w_down):
    def _A_ref(x, wqkv, wo):
        B, S, D = x.shape
        H = 32; Dh = D // H; W = 256
        qkv = (lambda x, *d: x.transpose(*d))((x @ wqkv).reshape(B, S, 3, H, Dh), 2, 0, 3, 1, 4)
        q, k, v = qkv[0], qkv[1], qkv[2]
        scores = jnp.einsum("bhqd,bhkd->bhqk", q, k) * (Dh ** -0.5)
        idx = jnp.arange(S)
        mask = (idx[:, None] - idx[None, :] >= 0) & (idx[:, None] - idx[None, :] < W)
        scores = jnp.where(mask[None, None], scores, -1e9)
        p = _softmax(scores, axis=-1)
        o = jnp.einsum("bhqk,bhkd->bhqd", p, v)
        return (lambda x, *d: x.transpose(*d))(o, 0, 2, 1, 3).reshape(B, S, D) @ wo

    def _B_ref(x, w_gate, w_up, w_down):
        g = _silu(x @ w_gate)
        u = x @ w_up
        return (g * u) @ w_down

    x = A_x
    h = x + _A_ref(_layernorm(x, axis=-1), A_wqkv, A_wo)
    h2 = h + _B_ref(_layernorm(h, axis=-1), B_w_gate, B_w_up, B_w_down)
    return h2
```

```python
import functools
import math

import jax
import jax.numpy as jnp
from jax import lax
from jax.experimental import pallas as pl
from jax.experimental.pallas import tpu as pltpu

H, DH, WIN, EPS = 32, 16, 256, 1e-5
QB = 128
TM = 256
G = 4
NEG = -1e30
PR, EPT, PAD = 16, 2, 8
PPOS, QSHARE, GAP = (0, 1, 2), 300, 512
HEAD, OPOS, UEND, LNEND, L1END, U0 = 14, 7, 5, 18, 5, 5
NE, DN, WPOS = 3, 3, 9
F32, BF16 = jnp.float32, jnp.bfloat16
NT = (((1,), (1,)), ((), ()))


def _ln(x):
    m = jnp.mean(x, axis=-1, keepdims=True)
    xc = x - m
    v = jnp.mean(xc * xc, axis=-1, keepdims=True)
    return xc * lax.rsqrt(v + EPS)


def _aligned(i, n):
    return i if isinstance(i, int) else pl.multiple_of(i, n)


def _load(ref, idx, start=0, size=None):
    size = ref.shape[-2] if size is None else size
    rows = pl.ds(_aligned(start // 2, 8), size // 2)
    return pltpu.bitcast(ref.bitcast(jnp.uint32)[(*idx, rows, slice(None))], BF16)


def _pack(x):
    return [pltpu.pack_elementwise([x[r:r + 8], x[r + 8:r + 16]], packed_dtype=BF16)
            for r in range(0, x.shape[0], 16)]


def _as_bf16(parts):
    return jnp.concatenate([pltpu.bitcast(p, BF16) for p in parts], axis=0)


class _Pace:
    def __init__(self, zero_ref):
        self.zero_ref, self.src, self.on = zero_ref, None, True

    def mark(self, result):
        self.src = result

    def hold(self, xs, frac):
        if self.src is None or not self.on:
            return xs
        i = int(frac * (self.src.shape[0] // 8))
        dep = pltpu.bitcast(self.src[8 * i:8 * i + 8, :128], jnp.uint32) & self.zero_ref[...]
        return [pltpu.bitcast(pltpu.bitcast(x, jnp.uint32) | dep, x.dtype) for x in xs]


class _Attn:
    def __init__(self, refs, qrow, q0, nkb, G, lg, sg, par):
        self.refs, self.qrow, self.q0, self.nkb, self.G = refs, qrow, q0, nkb, G
        self.lg, self.sg, self.par = lg, sg, par
        self.w = QB // G
        self.m, self.live, self.l, self.o = [None] * G, [None] * G, [None] * G, [None] * G

    def qk(self, j):
        q_ref, k_ref, _, _, s_ref, _, _, pace = self.refs
        G, w = self.G, self.w
        lane_h = lax.broadcasted_iota(jnp.int32, (w // 2, 128), 1) // DH
        qj = pltpu.bitcast(_load(q_ref[self.lg // 2], (self.lg % 2,), self.q0 + j * w, w), jnp.int32)
        qbd = jnp.concatenate(
            [jnp.where(lane_h == self.sg * G + (g - j) % G, qj, 0) for g in range(G)], axis=0)
        r0, r1 = max(j * w, (3 - self.nkb) * QB), j * w + WIN + w
        kw = _load(k_ref[self.lg // 2], (self.lg % 2,), self.q0 - WIN + r0, r1 - r0)
        s = lax.dot_general(kw, pltpu.bitcast(qbd, BF16), NT, preferred_element_type=F32)
        pace.mark(s)
        tri = (lax.broadcasted_iota(jnp.int32, (w, 128), 0)
               <= lax.broadcasted_iota(jnp.int32, (w, 128), 1) % w)
        near = s[j * w + WIN - r0:]
        pieces = [(j * w, jnp.where(tri, near, s[:w] if self.nkb == 3 else NEG))]
        lo = max(j * w + w, r0)
        if lo < WIN:
            pieces.append((lo, s[lo - r0:WIN - r0]))
        if j:
            pieces.append((0, s[WIN - r0:WIN - r0 + j * w]))
        for r, v in pieces:
            s_ref[self.par][j, pl.ds(r, v.shape[0]), :] = v
        allv = jnp.concatenate([v for _, v in pieces], axis=0)
        self.m[j] = jnp.broadcast_to(jnp.max(allv, axis=0, keepdims=True), (8, 128))
        self.live[j] = {r // 16 + t for r, v in pieces for t in range(v.shape[0] // 16)}

    def exp(self, r, frac):
        s_ref, p_ref, mask_ref, pace = self.refs[4:]
        G = self.G
        if not any(r in lv for lv in self.live):
            return
        n = G // len(frac)
        z, m = [], [v for i, f in enumerate(frac) for v in pace.hold(self.m[i * n:(i + 1) * n], f)]
        for j in range(G):
            if r in self.live[j]:
                e = [jnp.exp2(s_ref[self.par][j, pl.ds(16 * r + o, 8), :] - m[j]) for o in (0, 8)]
                self.l[j] = e[0] + e[1] if self.l[j] is None else self.l[j] + (e[0] + e[1])
                z.append(pltpu.pack_elementwise(e, packed_dtype=BF16))
            else:
                z.append(jnp.zeros((8, 128), jnp.uint32))
        for hh, v in enumerate(self.by_head(z)):
            if r >= 8:
                p_ref[self.par][hh, pl.ds(8 * r, 8), :] = v
            elif self.nkb < 3:
                p_ref[self.par][hh, pl.ds(8 * (r + 16), 8), :] = v
            else:
                near = v & mask_ref[hh, pl.ds(8 * r, 8), :]
                p_ref[self.par][hh, pl.ds(8 * r, 8), :] = v ^ near
                p_ref[self.par][hh, pl.ds(8 * (r + 16), 8), :] = near

    def by_head(self, z):
        G = self.G
        grp = lax.broadcasted_iota(jnp.int32, (8, 128), 1) // self.w
        b = 1
        while b < G:
            z = [jnp.where((grp & b) != 0, z[(n + b) % G], z[n]) for n in range(G)]
            b *= 2
        return [z[(-hh) % G] for hh in range(G)]

    def pv(self, b, heads):
        _, _, vt_ref, ot_ref, _, p_ref, _, _ = self.refs
        G = self.G
        if b < 3 - self.nkb:
            return
        sums = self.by_head(self.l) if b == 2 else None
        for hh in heads:
            head = self.lg * 8 + self.sg * G + hh
            p = pltpu.bitcast(p_ref[self.par][hh, pl.ds(b * 64, 64), :], BF16)
            vt = _load(vt_ref, (self.q0 // QB - 2 + b,), head * DH, DH)
            o = jnp.dot(vt, p, preferred_element_type=F32)
            o = self.o[hh] = o if self.o[hh] is None else o + self.o[hh]
            if b == 2:
                o = o * pl.reciprocal(jnp.sum(sums[hh], axis=0, keepdims=True))
                if hh:
                    o = pltpu.roll(o, (G - hh) * self.w, axis=1)
                ot_ref[self.qrow // QB, pl.ds(head * DH, DH), :] = o


def _init_masks(mask_ref, G):
    w = QB // G
    row = lax.broadcasted_iota(jnp.int32, (64, 128), 0)
    lane = lax.broadcasted_iota(jnp.int32, (64, 128), 1)
    key = (row // 8) * 16 + row % 8
    for hh in range(G):
        qry = (lane + (G - hh) * w) % QB
        bits = jnp.where(key <= qry, 0xFFFF, 0) | jnp.where(key + 8 <= qry, -0x10000, 0)
        mask_ref[hh] = pltpu.bitcast(bits, jnp.uint32)


def _attn_tasks(refs, blocks, G, fill, ppos, qshare):
    keys = [(qrow, q0, nkb, G, lg, sg)
            for (qrow, q0, nkb) in blocks for lg in range(4) for sg in range(8 // G)]
    groups = [_Attn(refs, *k, n % 2) for n, k in enumerate(keys)]
    n, P = len(groups), functools.partial
    total, done, spent, tasks = sum(c for c, _ in fill), 0, 0, []
    for t in range(n + 2):
        mine = []
        while done < len(fill) and spent + fill[done][0] / 2 <= total * (t + 1) / (n + 2):
            mine.append(fill[done])
            spent += fill[done][0]
            done += 1
        units, after, parts = [], {}, G // 4
        for h in range(parts):
            js = range(4 * h, 4 * h + 4)
            qk = [P(groups[t].qk, j) for j in js] if t < n else []
            sub = mine[len(mine) * h // parts:len(mine) * (h + 1) // parts]
            if t >= 2:
                for b in range(3):
                    after.setdefault(len(units) + min(ppos[b], len(sub)), []).append(P(groups[t - 2].pv, b, js))
            units += [(qshare, P(_run, qk))] + sub
        span, start, k = sum(c for c, _ in units), 0, 0
        for u, (c, f) in enumerate(units):
            tasks.append(f)
            while 1 <= t <= n and k < 16 and (k + 0.5) / 16 * span < start + c:
                at = [(k + (i + 0.5) / EPT) / 16 * span - start for i in range(EPT)]
                tasks.append(P(groups[t - 1].exp, k, [min(max(v / c, 0), 0.99) for v in at]))
                k += 1
            start += c
            tasks += after.get(u, [])
    return tasks


def _run(tasks):
    for f in tasks:
        f()


def _lhs_terms(a11, a12, a21, a22):
    return (a11 + a22, a21 + a22, a11, a22, a11 + a12, a21 - a11, a12 - a22)


def _rhs_terms(b11, b12, b21, b22):
    return (b11 + b22, b11, b12 - b22, b21 - b11, b22, b11 + b12, b21 + b22)


QKV_PAIRS = ((0, 4), (8, 10), (2, 6))
SUMMED = {0: 0, 2: 1, 3: 2, 5: 3, 6: 4}


def _strassen(prod, emit, ktiles=2):
    m = {}

    def step(i):
        m[i] = prod(i)
        if i == 3:
            emit(1, 0, m[1] + m[3])
        elif i == 6:
            emit(0, 0, m[0] + m[3] - m[4] + m[6])
        elif i == 2:
            emit(0, 1, m[2] + m[4])
        elif i == 5:
            emit(1, 1, m[0] - m[1] + m[2] + m[5])
    return [(64 * ktiles, functools.partial(step, i)) for i in (4, 1, 3, 0, 6, 2, 5)]


def _lanes(ref, idx, n):
    return jnp.concatenate([_load(ref, (*idx, l)) for l in range(n)], axis=1)


class _TileCopy:
    def __init__(self, src, dst, tiles, sem):
        self.copies = [pltpu.make_async_copy(src.at[:, pl.ds(n * 128, 128)], dst.at[n], sem) for n in tiles]

    def start(self):
        _run([c.start for c in self.copies])

    def wait(self):
        _run([c.wait for c in self.copies])


def _tiles(ref, first, n, start=0, size=None):
    return jnp.concatenate([_load(ref, (first + l,), start, size) for l in range(n)], axis=1)


def _kernel(x_hbm, wqkv_hbm, wo_hbm, wg_hbm, wu_hbm, wd_hbm, o_hbm,
            x_s, o_s, wqkv, wo, wg, wu, wd, bqkv, bo, bgu, bd, q0_s, q1_s, k0_s, k1_s, vt_s, ot_s, on_s, h_s, ao_s, ax_s, ah_s, ad_s,
            s0_s, s1_s, p0_s, p1_s, mask_s, zero_s, sems, osems):
    S, D = x_s.shape
    F = wg_hbm.shape[-1]
    NB, NC, HM, HD = S // TM, F // 256, TM // 2, D // 2
    P = functools.partial
    pace = _Pace(zero_s)
    q_s, k_s = (q0_s, q1_s), (k0_s, k1_s)
    refs = (q_s, k_s, vt_s, ot_s, (s0_s, s1_s), (p0_s, p1_s), mask_s, pace)

    def copy(n, src, dst, *idx):
        return pltpu.make_async_copy(src.at[idx], dst.at[idx], sems.at[n])

    cp_x0 = copy(0, x_hbm, x_s, pl.ds(0, TM))
    cp_x1 = copy(1, x_hbm, x_s, pl.ds(TM, TM))
    cp_x1b = copy(2, x_hbm, x_s, pl.ds(2 * TM, TM))
    cp_x2 = copy(3, x_hbm, x_s, pl.ds(3 * TM, S - 3 * TM))
    cp_qkv = [_TileCopy(wqkv_hbm, wqkv, range(4 * n, 4 * n + 4), sems.at[4 + n]) for n in range(3)]
    cp_wo = _TileCopy(wo_hbm, wo, range(4), sems.at[7])
    cp_wd = _TileCopy(wd_hbm, wd, range(4), sems.at[8])
    cp_gu = [[_TileCopy(src, dst, tiles, sems.at[9 + 2 * c + n])
              for n, (src, dst) in enumerate(((wg_hbm, wg), (wu_hbm, wu)))]
             for c, tiles in enumerate((range(2 * NE), range(2 * NE, 2 * NC)))]

    def rows(t, half=None):
        if half is None:
            return pl.ds(_aligned(t * TM, TM), TM)
        return pl.ds(_aligned(t * TM + half * HM, HM), HM)

    def out_copy(t):
        return pltpu.make_async_copy(o_s.at[rows(t)], o_hbm.at[rows(t)], osems.at[t])

    def put_terms(dst, idx, terms):
        for i, v in enumerate(terms):
            dst[(i, *idx)] = v.astype(BF16)

    def prep(dst, idx, srcs, frac):
        for n in (0, 3):
            v = pltpu.bitcast(srcs[n], jnp.uint32)
            srcs[n] = _as_bf16(pace.hold([v[r:r + 8] for r in range(0, v.shape[0], 8)], frac))
        terms = _rhs_terms(*[v.astype(F32) for v in srcs])
        for i, j in SUMMED.items():
            dst[(j, *idx)] = terms[i].astype(BF16)

    def rhs(i, sums, idx, b11, b22):
        return _lanes(sums, (SUMMED[i], *idx), 2) if i in SUMMED else (b11() if i == 1 else b22())

    def prep_qkv(c, l, r, frac):
        prep(bqkv, (c, l, pl.ds(r, PR)),
             [_load(wqkv, (n + l,), k + r, PR) for k in (0, HD) for n in QKV_PAIRS[c]], frac)

    def prep_gu(c, l, r, frac):
        prep(bgu, (c, l, pl.ds(r, PR)), [_load(w, (2 * c + l,), k + r, PR) for k in (0, HD) for w in (wg, wu)], frac)

    def prep_d(c, l, r, frac):
        prep(bd, (l, pl.ds(c * 128 + r, PR)),
             [_load(wd, (n + l,), c * 256 + k + r, PR) for k in (0, 128) for n in (0, 2)], frac)

    def put_ln(dst, load, r, frac):
        v = []
        for half in range(2):
            u = load(half * HM + r)
            head = jnp.concatenate(pace.hold([u[:8, :128], u[8:, :128]], frac), axis=0)
            v.append(_ln(jnp.concatenate([head, u[:, 128:]], axis=1)))
        for l in range(2):
            put_terms(dst, (l, pl.ds(r, 16)),
                      _lhs_terms(*[u[:, n + l * 128:n + (l + 1) * 128] for u in v for n in (0, HD)]))

    def put_qkv(t, half, col, r):
        for l in range(r.shape[1] // 128):
            n, lg = divmod(col // 128 + l, 4)
            v = r[:, l * 128:(l + 1) * 128]
            if n == 0:
                q_s[lg // 2][lg % 2, rows(t, half), :] = (v * (DH ** -0.5 * math.log2(math.e))).astype(BF16)
            elif n == 1:
                k_s[lg // 2][lg % 2, rows(t, half), :] = v.astype(BF16)
            else:
                vt_s[2 * t + half, pl.ds(lg * 128, 128), :] = _as_bf16(_pack(v)).T

    def dot(a, b):
        r = jnp.dot(a, b, preferred_element_type=F32)
        pace.mark(r)
        return r

    def qkv_tasks(t):
        tasks = []
        for c in range(3):
            tasks += _strassen(
                lambda i, c=c: dot(_lanes(ax_s, (i,), 2), rhs(
                    i, bqkv, (c,), lambda: _tiles(wqkv, QKV_PAIRS[c][0], 2, 0, HD),
                    lambda: _tiles(wqkv, QKV_PAIRS[c][1], 2, HD, HD))),
                lambda a, b, r, c=c: put_qkv(t, a, QKV_PAIRS[c][b] * 128, r))
        return tasks

    def ln1(t):
        return [P(put_ln, ax_s, lambda r: x_s[pl.ds(_aligned(t * TM + r, 16), 16), :].astype(F32), r)
                for r in range(0, HM, 16)]

    def ln2():
        return [P(put_ln, ah_s, lambda r: h_s[pl.ds(r, 16), :], r) for r in range(0, HM, 16)]

    def untranspose(b, lg, frac):
        on_s[lg, pl.ds(b * QB, QB), :] = ot_s[b, pl.ds(lg * 128, 128), :].T

    def o_terms(l, r, frac):
        put_terms(ao_s, (l, pl.ds(r, 64)),
                  _lhs_terms(*[on_s[n + l, pl.ds(b * HM + r, 64), :] for b in range(2) for n in (0, 2)]))

    untr0 = [P(untranspose, 0, lg) for lg in range(4)]
    untr = [f for l in range(2) for f in (
        [P(untranspose, 1, n + l) for n in (0, 2)] + [P(o_terms, l, r) for r in (0, 64)])]

    def prep_o(l, r, frac):
        prep(bo, (l, pl.ds(r, PR)), [_load(wo, (n + l,), k + r, PR) for k in (0, HD) for n in (0, 2)], frac)

    def oproj_tasks(t):
        def emit(a, b, r):
            cols = pl.ds(b * HD, HD)
            h_s[pl.ds(a * HM, HM), cols] = x_s[rows(t, a), cols].astype(F32) + r
        return _strassen(
            lambda i: dot(_lanes(ao_s, (i,), 2), rhs(
                i, bo, (), lambda: _tiles(wo, 0, 2, 0, HD), lambda: _tiles(wo, 2, 2, HD, HD))), emit)

    def ffn_tasks(t):
        tasks = []
        for c in range(NC):
            st = {}

            def emit(a, b, r, c=c, st=st):
                if b == 0:
                    hg = 0.5 * r
                    st[a] = hg + hg * jnp.tanh(hg)
                    return
                st[a] = st[a] * r
                if a == 1:
                    quad = [st[i][:, l * 128:(l + 1) * 128] for i in range(2) for l in range(2)]
                    put_terms(ad_s, (c,), _lhs_terms(*quad))
            tasks += _strassen(
                lambda i, c=c: dot(_lanes(ah_s, (i,), 2), rhs(
                    i, bgu, (c,), lambda: _tiles(wg, 2 * c, 2, 0, HD),
                    lambda: _tiles(wu, 2 * c, 2, HD, HD))), emit)

        def down(i):
            lhs = jnp.concatenate([_load(ad_s, (i, k)) for k in range(NC)], axis=1)
            if i in SUMMED:
                w = [_load(bd, (SUMMED[i], l)) for l in range(2)]
                return dot(lhs, jnp.concatenate(w, axis=1))
            n = 0 if i == 1 else 1
            w = [_tiles(wd, 2 * n, 2, c * 256 + n * 128, 128) for c in range(NC)]
            return dot(lhs, jnp.concatenate(w, axis=0))

        def store(a, b, r):
            cols = pl.ds(b * HD, HD)
            o_s[rows(t, a), cols] = (h_s[pl.ds(a * HM, HM), cols] + r).astype(o_s.dtype)
        return tasks + _strassen(down, store, NC)

    def attach(units, extra, lo, hi):
        for n, g in enumerate(extra):
            u, frac = divmod((n + 0.5) * (hi - lo) / len(extra), 1)
            cost, f = units[lo + int(u)]
            units[lo + int(u)] = (cost, P(_run, [f, P(g, frac)]))

    def attention(t, fill, nkb=(3, 3)):
        pace.mark(None)
        _run(_attn_tasks(refs, [(b * QB, t * TM + b * QB, nkb[b]) for b in range(2)], G, fill, PPOS, QSHARE))

    def start(*cps):
        return [lambda _: _run([c.start for c in cps])]

    def wait(*cps):
        return [lambda _: _run([c.wait for c in cps])]

    _run([c.start for c in (cp_x0, cp_qkv[0], cp_qkv[1])])
    _init_masks(mask_s, G)
    zero_s[...] = jnp.zeros_like(zero_s)
    cp_x0.wait()
    _run([c.start for c in (cp_qkv[2], cp_x1)])
    xn = _ln(x_s[rows(0), :].astype(F32)).astype(BF16)
    cp_qkv[0].wait()

    def proj0(n):
        r = dot(xn, _load(wqkv, (n,)))
        for half in range(2):
            put_qkv(0, half, n * 128, r[half * HM:(half + 1) * HM])
    qt = [(256, P(proj0, n)) for n in range(12)]
    preps = [[P(prep_qkv, c, l, r) for l in range(2) for r in range(0, HD, PR)] for c in range(3)]
    gu = [[P(prep_gu, c, l, r) for l in range(2) for r in range(0, HD, PR)] for c in range(NC)]
    attach(qt, wait(cp_qkv[1]) + start(*cp_gu[0]), 3, 4)
    attach(qt, preps[0], 4, 7)
    attach(qt, wait(cp_qkv[2], cp_x1) + start(cp_wo, *cp_gu[1], cp_wd, cp_x1b), 7, 8)
    attach(qt, ln1(1) + preps[1], 8, 12)
    _run([f for _, f in qt[:8]])
    q1 = qkv_tasks(1)
    po = [P(prep_o, l, r) for l in range(2) for r in range(0, HD, PR)]
    attach(q1, preps[2], 0, WPOS)
    attach(q1, wait(*cp_gu[0], cp_wo) + start(cp_x2), WPOS - 1, WPOS)
    attach(q1, po + sum(gu[:NE], []), WPOS, 21)
    attach(q1, untr0, 17, 21)
    attention(0, qt[8:] + q1, (1, 2))

    ot, ft = oproj_tasks(0), ffn_tasks(0)
    pace.mark(None)
    _run([P(f, 0) for f in untr])
    attach(ot, ln2(), 6, 7)
    w2 = 7 * (NE - 1) + 2
    attach(ft, wait(*cp_gu[1], cp_wd, cp_x1b), w2 - 1, w2)
    dn = [P(prep_d, c, l, r) for c in range(NC) for l in range(2) for r in range(0, 128, PR)]
    for c in range(NE, NC):
        attach(ft, gu[c] + dn[DN * (c - NE):DN * (c - NE + 1)], 7 * c - 5, 7 * c + 2)
    rest = dn[DN * (NC - NE):]
    attach(ft, rest[:len(rest) // 2], 7 * NC - 5, 7 * NC)
    attach(ft, rest[len(rest) // 2:], 7 * NC, 7 * NC + 1)
    attach(ft, ln1(2), 7 * NC + 2, 7 * NC + 6)
    attach(ft, untr0, 7 * NC + U0, 7 * NC + 7)
    attention(1, ot + [(GAP, lambda: None)] + ft)
    out_copy(0).start()
    cp_x2.wait()

    def body(t, carry):
        pace.mark(None)
        qt, ft = qkv_tasks(t), ffn_tasks(t - 1)
        attach(qt, untr, 0, UEND)
        attach(qt, ln2(), OPOS, LNEND)
        attach(ft, ln1(jnp.minimum(t + 1, NB - 1)), 7 * NC, 7 * NC + L1END)
        attach(ft, untr0, 7 * NC + U0, 7 * NC + 7)
        units = qt[:OPOS] + oproj_tasks(t - 1) + qt[OPOS:] + ft
        _run([f for _, f in units[:HEAD]])
        attention(t, units[HEAD:])
        out_copy(t - 1).start()
        return carry

    lax.fori_loop(2, NB, body, 0)
    pace.mark(None)
    _run([P(f, 0) for f in untr] + [f for _, f in oproj_tasks(NB - 1)])
    pace.mark(None)
    last = [pltpu.make_async_copy(o_s.at[rows(NB - 1, n)], o_hbm.at[rows(NB - 1, n)], osems.at[NB - 1 + n])
            for n in range(2)]
    ft = [f for _, f in ffn_tasks(NB - 1)]
    _run([P(f, 0) for f in ln2()] + ft[:-1] + [last[0].start] + ft[-1:])
    last[1].start()
    _run([out_copy(t).wait for t in range(NB - 1)] + [c.wait for c in last])


@jax.jit
def pallas_sequential_preLN__sliding_block__swiglu_ffn__prompt_kernel(
        A_x, A_wqkv, A_wo, B_x, B_w_gate, B_w_up, B_w_down):
    del B_x
    B, S, D = A_x.shape
    F = B_w_gate.shape[1]
    hbm = pl.BlockSpec(memory_space=pl.ANY)
    vmem = pltpu.VMEM
    out = pl.pallas_call(
        _kernel,
        in_specs=[hbm] * 6,
        out_specs=hbm,
        out_shape=jax.ShapeDtypeStruct((S, D), A_x.dtype),
        scratch_shapes=[
            vmem((S, D), BF16), vmem((S, D), BF16),
            vmem((3 * D // 128, D, 128), BF16), vmem((D // 128, D, 128), BF16),
            vmem((F // 128, D, 128), BF16), vmem((F // 128, D, 128), BF16), vmem((D // 128, F, 128), BF16),
            vmem((5, 3, 2, D // 2, 128), BF16), vmem((5, 2, D // 2, 128), BF16), vmem((5, F // 256, 2, D // 2, 128), BF16),
            vmem((5, 2, F // 2, 128), BF16),
            *[vmem((2, S, 128), BF16)] * 4,
            vmem((S // QB, D, QB), BF16), vmem((TM // QB, D, QB), F32), vmem((4, TM, 128), F32), vmem((TM, D), F32),
            vmem((7, 2, TM // 2, 128), BF16), vmem((7, 2, TM // 2, 128), BF16),
            vmem((7, 2, TM // 2, 128), BF16),
            vmem((7, F // 256, TM // 2, 128), BF16),
            vmem((G, WIN + PAD, 128), F32), vmem((G, WIN + PAD, 128), F32),
            vmem((G, 192 + PAD, 128), jnp.uint32), vmem((G, 192 + PAD, 128), jnp.uint32),
            vmem((G, 64, 128), jnp.uint32), vmem((8, 128), jnp.uint32),
            pltpu.SemaphoreType.DMA((13,)), pltpu.SemaphoreType.DMA((S // TM + 1,)),
        ],
        compiler_params=pltpu.CompilerParams(
            vmem_limit_bytes=100 * 2**20, flags={"XLA_TPU_EVENLY_DISTRIBUTE_CRITICAL_NODES": True}),
    )(A_x.reshape(S, D), A_wqkv, A_wo, B_w_gate, B_w_up, B_w_down)
    return out.reshape(B, S, D)
```

```python
import functools
import math

import jax
import jax.numpy as jnp
from jax import lax
from jax.experimental import pallas as pl
from jax.experimental.pallas import tpu as pltpu

DH, WIN, EPS = 16, 256, 1e-5
QB = 128
TM = 256
G = 4
NEG = -1e30
PR, EPT, PAD = 16, 4, 8
PPOS, QSHARE, GAP = (0, 1, 2), 300, 512
HEAD, OPOS, UEND, LNEND, L1END, U0 = 16, 7, 5, 18, 5, 5
NE, DN, WPOS = 3, 3, 9
F32, BF16 = jnp.float32, jnp.bfloat16
NT = (((1,), (1,)), ((), ()))


def _ln(x):
    m = jnp.mean(x, axis=-1, keepdims=True)
    xc = x - m
    v = jnp.mean(xc * xc, axis=-1, keepdims=True)
    return xc * lax.rsqrt(v + EPS)


def _aligned(i, n):
    return i if isinstance(i, int) else pl.multiple_of(i, n)


def _load(ref, idx, start=0, size=None):
    size = ref.shape[-2] if size is None else size
    rows = pl.ds(_aligned(start // 2, 8), size // 2)
    return pltpu.bitcast(ref.bitcast(jnp.uint32)[(*idx, rows, slice(None))], BF16)


def _as_bf16(parts):
    return jnp.concatenate([pltpu.bitcast(p, BF16) for p in parts], axis=0)


class _Pace:
    def __init__(self, zero_ref):
        self.zero_ref, self.src, self.on = zero_ref, None, True

    def mark(self, result):
        self.src = result

    def hold(self, xs, frac):
        if self.src is None or not self.on:
            return xs
        i = int(frac * (self.src.shape[0] // 8))
        dep = pltpu.bitcast(self.src[8 * i:8 * i + 8, :128], jnp.uint32) & self.zero_ref[...]
        return [pltpu.bitcast(pltpu.bitcast(x, jnp.uint32) | dep, x.dtype) for x in xs]


class _Attn:
    def __init__(self, refs, qrow, q0, nkb, G, lg, sg, par):
        self.refs, self.qrow, self.q0, self.nkb, self.G = refs, qrow, q0, nkb, G
        self.lg, self.sg, self.par = lg, sg, par
        self.w = QB // G
        self.m, self.live, self.l, self.o = [None] * G, [None] * G, [None] * G, [None] * G

    def qk(self, j):
        q_ref, k_ref, _, _, s_ref, _, _, pace = self.refs
        G, w = self.G, self.w
        lane_h = lax.broadcasted_iota(jnp.int32, (w // 2, 128), 1) // DH
        qj = pltpu.bitcast(_load(q_ref[self.lg // 2], (self.lg % 2,), self.q0 + j * w, w), jnp.int32)
        qbd = jnp.concatenate(
            [jnp.where(lane_h == self.sg * G + (g - j) % G, qj, 0) for g in range(G)], axis=0)
        r0, r1 = max(j * w, (3 - self.nkb) * QB), j * w + WIN + w
        kw = _load(k_ref[self.lg // 2], (self.lg % 2,), self.q0 - WIN + r0, r1 - r0)
        s = lax.dot_general(kw, pltpu.bitcast(qbd, BF16), NT, preferred_element_type=F32)
        pace.mark(s)
        tri = (lax.broadcasted_iota(jnp.int32, (w, 128), 0)
               <= lax.broadcasted_iota(jnp.int32, (w, 128), 1) % w)
        near = s[j * w + WIN - r0:]
        pieces = [(j * w, jnp.where(tri, near, s[:w] if self.nkb == 3 else NEG))]
        lo = max(j * w + w, r0)
        if lo < WIN:
            pieces.append((lo, s[lo - r0:WIN - r0]))
        if j:
            pieces.append((0, s[WIN - r0:WIN - r0 + j * w]))
        for r, v in pieces:
            s_ref[self.par][j, pl.ds(r, v.shape[0]), :] = v
        allv = jnp.concatenate([v for _, v in pieces], axis=0)
        self.m[j] = jnp.broadcast_to(jnp.max(allv, axis=0, keepdims=True), (8, 128))
        self.live[j] = {r // 16 + t for r, v in pieces for t in range(v.shape[0] // 16)}

    def exp(self, r, frac):
        s_ref, p_ref, _, pace = self.refs[4:]
        G = self.G
        if not any(r in lv for lv in self.live):
            return
        n = G // len(frac)
        m = [v for i, f in enumerate(frac) for v in pace.hold(self.m[i * n:(i + 1) * n], f)]
        for j in range(G):
            if r in self.live[j]:
                e = [jnp.exp2(s_ref[self.par][j, pl.ds(16 * r + o, 8), :] - m[j]) for o in (0, 8)]
                self.l[j] = e[0] + e[1] if self.l[j] is None else self.l[j] + (e[0] + e[1])
                p = jnp.concatenate(e, axis=0).astype(BF16)
            else:
                p = jnp.zeros((16, 128), BF16)
            p_ref[self.par][j, pl.ds(16 * r, 16), :] = p

    def by_head(self, z):
        G = self.G
        grp = lax.broadcasted_iota(jnp.int32, (8, 128), 1) // self.w
        b = 1
        while b < G:
            z = [jnp.where((grp & b) != 0, z[(n + b) % G], z[n]) for n in range(G)]
            b *= 2
        return [z[(-hh) % G] for hh in range(G)]

    def pv(self, b, heads):
        _, _, vt_ref, ot_ref, _, p_ref, mask_ref, _ = self.refs
        G = self.G
        if b < 3 - self.nkb:
            return
        sums = self.by_head(self.l) if b == 2 else None
        packed = p_ref[self.par].bitcast(jnp.uint32)
        rows = [self.by_head([packed[j, pl.ds(8 * r, 8), :] for j in range(G)])
                for r in (range(8, 16) if b == 1 else range(8))]
        for hh in heads:
            head = self.lg * 8 + self.sg * G + hh
            p = [row[hh] for row in rows]
            if b != 1 and self.nkb == 3:
                near = [v & mask_ref[hh, pl.ds(8 * r, 8), :] for r, v in enumerate(p)]
                p = near if b == 2 else [v ^ n for v, n in zip(p, near)]
            p = _as_bf16(p)
            vt = _load(vt_ref, (self.q0 // QB - 2 + b,), head * DH, DH)
            o = jnp.dot(vt, p, preferred_element_type=F32)
            o = self.o[hh] = o if self.o[hh] is None else o + self.o[hh]
            if b == 2:
                o = o * pl.reciprocal(jnp.sum(sums[hh], axis=0, keepdims=True))
                if hh:
                    o = pltpu.roll(o, (G - hh) * self.w, axis=1)
                ot_ref[self.qrow // QB, pl.ds(head * DH, DH), :] = o


def _init_masks(mask_ref, G):
    w = QB // G
    row = lax.broadcasted_iota(jnp.int32, (64, 128), 0)
    lane = lax.broadcasted_iota(jnp.int32, (64, 128), 1)
    key = 2 * row
    for hh in range(G):
        qry = (lane + (G - hh) * w) % QB
        bits = jnp.where(key <= qry, 0xFFFF, 0) | jnp.where(key + 1 <= qry, -0x10000, 0)
        mask_ref[hh] = pltpu.bitcast(bits, jnp.uint32)


def _attn_tasks(refs, blocks, G, fill, ppos, qshare):
    keys = [(qrow, q0, nkb, G, lg, sg)
            for (qrow, q0, nkb) in blocks for lg in range(4) for sg in range(8 // G)]
    groups = [_Attn(refs, *k, n % 2) for n, k in enumerate(keys)]
    n, P = len(groups), functools.partial
    total, done, spent, tasks = sum(c for c, _ in fill), 0, 0, []
    for t in range(n + 2):
        mine = []
        while done < len(fill) and spent + fill[done][0] / 2 <= total * (t + 1) / (n + 2):
            mine.append(fill[done])
            spent += fill[done][0]
            done += 1
        units, after, parts = [], {}, G // 4
        for h in range(parts):
            js = range(4 * h, 4 * h + 4)
            qk = [P(groups[t].qk, j) for j in js] if t < n else []
            sub = mine[len(mine) * h // parts:len(mine) * (h + 1) // parts]
            if t >= 2:
                for b in range(3):
                    after.setdefault(len(units) + min(ppos[b], len(sub)), []).append(P(groups[t - 2].pv, b, js))
            units += [(qshare, P(_run, qk))] + sub
        span, start, k = sum(c for c, _ in units), 0, 0
        for u, (c, f) in enumerate(units):
            tasks.append(f)
            while 1 <= t <= n and k < 16 and (k + 0.5) / 16 * span < start + c:
                at = [(k + (i + 0.5) / EPT) / 16 * span - start for i in range(EPT)]
                tasks.append(P(groups[t - 1].exp, k, [min(max(v / c, 0), 0.99) for v in at]))
                k += 1
            start += c
            tasks += after.get(u, [])
    return tasks


def _run(tasks):
    for f in tasks:
        f()


def _lhs_terms(a11, a12, a21, a22):
    return (a11 + a22, a21 + a22, a11, a22, a11 + a12, a21 - a11, a12 - a22)


def _rhs_terms(b11, b12, b21, b22):
    return (b11 + b22, b11, b12 - b22, b21 - b11, b22, b11 + b12, b21 + b22)


QKV_PAIRS = ((0, 4), (8, 10), (2, 6))
SUMMED = {0: 0, 2: 1, 3: 2, 5: 3, 6: 4}


def _strassen(prod, emit, ktiles=2):
    m = {}

    def step(i):
        m[i] = prod(i)
        if i == 3:
            emit(1, 0, m[1] + m[3])
        elif i == 6:
            emit(0, 0, m[0] + m[3] - m[4] + m[6])
        elif i == 2:
            emit(0, 1, m[2] + m[4])
        elif i == 5:
            emit(1, 1, m[0] - m[1] + m[2] + m[5])
    return [(64 * ktiles, functools.partial(step, i)) for i in (4, 1, 3, 0, 6, 2, 5)]


def _lanes(ref, idx, n):
    return jnp.concatenate([_load(ref, (*idx, l)) for l in range(n)], axis=1)


class _TileCopy:
    def __init__(self, src, dst, tiles, sem):
        self.copies = [pltpu.make_async_copy(src.at[:, pl.ds(n * 128, 128)], dst.at[n], sem) for n in tiles]

    def start(self):
        _run([c.start for c in self.copies])

    def wait(self):
        _run([c.wait for c in self.copies])


def _tiles(ref, first, n, start=0, size=None):
    return jnp.concatenate([_load(ref, (first + l,), start, size) for l in range(n)], axis=1)


def _kernel(x_hbm, wqkv_hbm, wo_hbm, wg_hbm, wu_hbm, wd_hbm, o_hbm,
            x_s, o_s, wqkv, wo, wg, wu, wd, bqkv, bo, bgu, bd, q0_s, q1_s, k0_s, k1_s, vt_s, ot_s, on_s, h_s, ao_s, ax_s, ah_s, ad_s,
            s0_s, s1_s, p0_s, p1_s, mask_s, zero_s, sems, osems):
    S, D = x_s.shape
    F = wg_hbm.shape[-1]
    NB, NC, HM, HD = S // TM, F // 256, TM // 2, D // 2
    P = functools.partial
    pace = _Pace(zero_s)
    q_s, k_s = (q0_s, q1_s), (k0_s, k1_s)
    refs = (q_s, k_s, vt_s, ot_s, (s0_s, s1_s), (p0_s, p1_s), mask_s, pace)

    def copy(n, src, dst, *idx):
        return pltpu.make_async_copy(src.at[idx], dst.at[idx], sems.at[n])

    cp_x0 = copy(0, x_hbm, x_s, pl.ds(0, TM))
    cp_x1 = copy(1, x_hbm, x_s, pl.ds(TM, TM))
    cp_x1b = copy(2, x_hbm, x_s, pl.ds(2 * TM, TM))
    cp_x2 = copy(3, x_hbm, x_s, pl.ds(3 * TM, S - 3 * TM))
    cp_qkv = [_TileCopy(wqkv_hbm, wqkv, range(4 * n, 4 * n + 4), sems.at[4 + n]) for n in range(3)]
    cp_wo = _TileCopy(wo_hbm, wo, range(4), sems.at[7])
    cp_wd = _TileCopy(wd_hbm, wd, range(4), sems.at[8])
    cp_gu = [[_TileCopy(src, dst, tiles, sems.at[9 + 2 * c + n])
              for n, (src, dst) in enumerate(((wg_hbm, wg), (wu_hbm, wu)))]
             for c, tiles in enumerate((range(2 * NE), range(2 * NE, 2 * NC)))]

    def rows(t, half=None):
        if half is None:
            return pl.ds(_aligned(t * TM, TM), TM)
        return pl.ds(_aligned(t * TM + half * HM, HM), HM)

    def out_copy(t):
        return pltpu.make_async_copy(o_s.at[rows(t)], o_hbm.at[rows(t)], osems.at[t])

    def put_terms(dst, idx, terms):
        for i, v in enumerate(terms):
            dst[(i, *idx)] = v.astype(BF16)

    def prep(dst, idx, srcs, frac):
        for n in (0, 3):
            v = pltpu.bitcast(srcs[n], jnp.uint32)
            srcs[n] = _as_bf16(pace.hold([v[r:r + 8] for r in range(0, v.shape[0], 8)], frac))
        terms = _rhs_terms(*[v.astype(F32) for v in srcs])
        for i, j in SUMMED.items():
            dst[(j, *idx)] = terms[i].astype(BF16)

    def rhs(i, sums, idx, b11, b22):
        return _lanes(sums, (SUMMED[i], *idx), 2) if i in SUMMED else (b11() if i == 1 else b22())

    def prep_qkv(c, l, r, frac):
        prep(bqkv, (c, l, pl.ds(r, PR)),
             [_load(wqkv, (n + l,), k + r, PR) for k in (0, HD) for n in QKV_PAIRS[c]], frac)

    def prep_gu(c, l, r, frac):
        prep(bgu, (c, l, pl.ds(r, PR)), [_load(w, (2 * c + l,), k + r, PR) for k in (0, HD) for w in (wg, wu)], frac)

    def prep_d(c, l, r, frac):
        prep(bd, (l, pl.ds(c * 128 + r, PR)),
             [_load(wd, (n + l,), c * 256 + k + r, PR) for k in (0, 128) for n in (0, 2)], frac)

    def put_ln(dst, load, r, frac):
        v = []
        for half in range(2):
            u = load(half * HM + r)
            head = jnp.concatenate(pace.hold([u[:8, :128], u[8:, :128]], frac), axis=0)
            v.append(_ln(jnp.concatenate([head, u[:, 128:]], axis=1)))
        for l in range(2):
            put_terms(dst, (l, pl.ds(r, 16)),
                      _lhs_terms(*[u[:, n + l * 128:n + (l + 1) * 128] for u in v for n in (0, HD)]))

    def put_qkv(t, half, col, r):
        for l in range(r.shape[1] // 128):
            n, lg = divmod(col // 128 + l, 4)
            v = r[:, l * 128:(l + 1) * 128]
            if n == 0:
                q_s[lg // 2][lg % 2, rows(t, half), :] = (v * (DH ** -0.5 * math.log2(math.e))).astype(BF16)
            elif n == 1:
                k_s[lg // 2][lg % 2, rows(t, half), :] = v.astype(BF16)
            else:
                vt_s[2 * t + half, pl.ds(lg * 128, 128), :] = v.astype(BF16).T

    def dot(a, b):
        r = jnp.dot(a, b, preferred_element_type=F32)
        pace.mark(r)
        return r

    def qkv_tasks(t):
        tasks = []
        for c in range(3):
            tasks += _strassen(
                lambda i, c=c: dot(_lanes(ax_s, (i,), 2), rhs(
                    i, bqkv, (c,), lambda: _tiles(wqkv, QKV_PAIRS[c][0], 2, 0, HD),
                    lambda: _tiles(wqkv, QKV_PAIRS[c][1], 2, HD, HD))),
                lambda a, b, r, c=c: put_qkv(t, a, QKV_PAIRS[c][b] * 128, r))
        return tasks

    def ln1(t):
        return [P(put_ln, ax_s, lambda r: x_s[pl.ds(_aligned(t * TM + r, 16), 16), :].astype(F32), r)
                for r in range(0, HM, 16)]

    def ln2():
        return [P(put_ln, ah_s, lambda r: h_s[pl.ds(r, 16), :], r) for r in range(0, HM, 16)]

    def untranspose(b, lg, frac):
        on_s[lg, pl.ds(b * QB, QB), :] = ot_s[b, pl.ds(lg * 128, 128), :].T

    def o_terms(l, r, frac):
        put_terms(ao_s, (l, pl.ds(r, 64)),
                  _lhs_terms(*[on_s[n + l, pl.ds(b * HM + r, 64), :] for b in range(2) for n in (0, 2)]))

    untr0 = [P(untranspose, 0, lg) for lg in range(4)]
    untr = [f for l in range(2) for f in (
        [P(untranspose, 1, n + l) for n in (0, 2)] + [P(o_terms, l, r) for r in (0, 64)])]

    def prep_o(l, r, frac):
        prep(bo, (l, pl.ds(r, PR)), [_load(wo, (n + l,), k + r, PR) for k in (0, HD) for n in (0, 2)], frac)

    def oproj_tasks(t):
        def emit(a, b, r):
            cols = pl.ds(b * HD, HD)
            h_s[pl.ds(a * HM, HM), cols] = x_s[rows(t, a), cols].astype(F32) + r
        return _strassen(
            lambda i: dot(_lanes(ao_s, (i,), 2), rhs(
                i, bo, (), lambda: _tiles(wo, 0, 2, 0, HD), lambda: _tiles(wo, 2, 2, HD, HD))), emit)

    def ffn_tasks(t):
        tasks = []
        for c in range(NC):
            st = {}

            def emit(a, b, r, c=c, st=st):
                if b == 0:
                    hg = 0.5 * r
                    st[a] = hg + hg * jnp.tanh(hg)
                    return
                st[a] = st[a] * r
                if a == 1:
                    quad = [st[i][:, l * 128:(l + 1) * 128] for i in range(2) for l in range(2)]
                    put_terms(ad_s, (c,), _lhs_terms(*quad))
            tasks += _strassen(
                lambda i, c=c: dot(_lanes(ah_s, (i,), 2), rhs(
                    i, bgu, (c,), lambda: _tiles(wg, 2 * c, 2, 0, HD),
                    lambda: _tiles(wu, 2 * c, 2, HD, HD))), emit)

        def down(i):
            lhs = jnp.concatenate([_load(ad_s, (i, k)) for k in range(NC)], axis=1)
            if i in SUMMED:
                w = [_load(bd, (SUMMED[i], l)) for l in range(2)]
                return dot(lhs, jnp.concatenate(w, axis=1))
            n = 0 if i == 1 else 1
            w = [_tiles(wd, 2 * n, 2, c * 256 + n * 128, 128) for c in range(NC)]
            return dot(lhs, jnp.concatenate(w, axis=0))

        def store(a, b, r):
            cols = pl.ds(b * HD, HD)
            o_s[rows(t, a), cols] = (h_s[pl.ds(a * HM, HM), cols] + r).astype(o_s.dtype)
        return tasks + _strassen(down, store, NC)

    def attach(units, extra, lo, hi):
        for n, g in enumerate(extra):
            u, frac = divmod((n + 0.5) * (hi - lo) / len(extra), 1)
            cost, f = units[lo + int(u)]
            units[lo + int(u)] = (cost, P(_run, [f, P(g, frac)]))

    def attention(t, fill, nkb=(3, 3)):
        pace.mark(None)
        _run(_attn_tasks(refs, [(b * QB, t * TM + b * QB, nkb[b]) for b in range(2)], G, fill, PPOS, QSHARE))

    def start(*cps):
        return [lambda _: _run([c.start for c in cps])]

    def wait(*cps):
        return [lambda _: _run([c.wait for c in cps])]

    _run([c.start for c in (cp_x0, cp_qkv[0], cp_qkv[1])])
    _init_masks(mask_s, G)
    zero_s[...] = jnp.zeros_like(zero_s)
    cp_x0.wait()
    _run([c.start for c in (cp_qkv[2], cp_x1)])
    xn = _ln(x_s[rows(0), :].astype(F32)).astype(BF16)
    cp_qkv[0].wait()

    def proj0(n):
        r = dot(xn, _load(wqkv, (n,)))
        for half in range(2):
            put_qkv(0, half, n * 128, r[half * HM:(half + 1) * HM])
    qt = [(256, P(proj0, n)) for n in range(12)]
    preps = [[P(prep_qkv, c, l, r) for l in range(2) for r in range(0, HD, PR)] for c in range(3)]
    gu = [[P(prep_gu, c, l, r) for l in range(2) for r in range(0, HD, PR)] for c in range(NC)]
    attach(qt, wait(cp_qkv[1]) + start(*cp_gu[0]), 3, 4)
    attach(qt, preps[0], 4, 7)
    attach(qt, wait(cp_qkv[2], cp_x1) + start(cp_wo, *cp_gu[1], cp_wd, cp_x1b), 7, 8)
    attach(qt, ln1(1) + preps[1], 8, 12)
    _run([f for _, f in qt[:8]])
    q1 = qkv_tasks(1)
    po = [P(prep_o, l, r) for l in range(2) for r in range(0, HD, PR)]
    attach(q1, preps[2], 0, WPOS)
    attach(q1, wait(*cp_gu[0], cp_wo) + start(cp_x2), WPOS - 1, WPOS)
    attach(q1, po + sum(gu[:NE], []), WPOS, 21)
    attach(q1, untr0, 17, 21)
    attention(0, qt[8:] + q1, (1, 2))

    ot, ft = oproj_tasks(0), ffn_tasks(0)
    pace.mark(None)
    _run([P(f, 0) for f in untr])
    attach(ot, ln2(), 6, 7)
    w2 = 7 * (NE - 1) + 2
    attach(ft, wait(*cp_gu[1], cp_wd, cp_x1b), w2 - 1, w2)
    dn = [P(prep_d, c, l, r) for c in range(NC) for l in range(2) for r in range(0, 128, PR)]
    for c in range(NE, NC):
        attach(ft, gu[c] + dn[DN * (c - NE):DN * (c - NE + 1)], 7 * c - 5, 7 * c + 2)
    rest = dn[DN * (NC - NE):]
    attach(ft, rest[:len(rest) // 2], 7 * NC - 5, 7 * NC)
    attach(ft, rest[len(rest) // 2:], 7 * NC, 7 * NC + 1)
    attach(ft, ln1(2), 7 * NC + 2, 7 * NC + 6)
    attach(ft, untr0, 7 * NC + U0, 7 * NC + 7)
    attention(1, ot + [(GAP, lambda: None)] + ft)
    out_copy(0).start()
    cp_x2.wait()

    def body(t, carry):
        pace.mark(None)
        qt, ft = qkv_tasks(t), ffn_tasks(t - 1)
        attach(qt, untr, 0, UEND)
        attach(qt, ln2(), OPOS, LNEND)
        attach(ft, ln1(jnp.minimum(t + 1, NB - 1)), 7 * NC, 7 * NC + L1END)
        attach(ft, untr0, 7 * NC + U0, 7 * NC + 7)
        units = qt[:OPOS] + oproj_tasks(t - 1) + qt[OPOS:] + ft
        _run([f for _, f in units[:HEAD]])
        attention(t, units[HEAD:])
        out_copy(t - 1).start()
        return carry

    lax.fori_loop(2, NB, body, 0)
    pace.mark(None)
    _run([P(f, 0) for f in untr] + [f for _, f in oproj_tasks(NB - 1)])
    pace.mark(None)
    last = [pltpu.make_async_copy(o_s.at[rows(NB - 1, n)], o_hbm.at[rows(NB - 1, n)], osems.at[NB - 1 + n])
            for n in range(2)]
    ft = [f for _, f in ffn_tasks(NB - 1)]
    _run([P(f, 0) for f in ln2()] + ft[:-1] + [last[0].start] + ft[-1:])
    last[1].start()
    _run([out_copy(t).wait for t in range(NB - 1)] + [c.wait for c in last])


@jax.jit
def pallas_sequential_preLN__sliding_block__swiglu_ffn__prompt_kernel(
        A_x, A_wqkv, A_wo, B_x, B_w_gate, B_w_up, B_w_down):
    del B_x
    B, S, D = A_x.shape
    F = B_w_gate.shape[1]
    hbm = pl.BlockSpec(memory_space=pl.ANY)
    vmem = pltpu.VMEM
    out = pl.pallas_call(
        _kernel,
        in_specs=[hbm] * 6,
        out_specs=hbm,
        out_shape=jax.ShapeDtypeStruct((S, D), A_x.dtype),
        scratch_shapes=[
            vmem((S, D), BF16), vmem((S, D), BF16),
            vmem((3 * D // 128, D, 128), BF16), vmem((D // 128, D, 128), BF16),
            vmem((F // 128, D, 128), BF16), vmem((F // 128, D, 128), BF16), vmem((D // 128, F, 128), BF16),
            vmem((5, 3, 2, D // 2, 128), BF16), vmem((5, 2, D // 2, 128), BF16), vmem((5, F // 256, 2, D // 2, 128), BF16),
            vmem((5, 2, F // 2, 128), BF16),
            *[vmem((2, S, 128), BF16)] * 4,
            vmem((S // QB, D, QB), BF16), vmem((TM // QB, D, QB), F32), vmem((4, TM, 128), F32), vmem((TM, D), F32),
            vmem((7, 2, TM // 2, 128), BF16), vmem((7, 2, TM // 2, 128), BF16),
            vmem((7, 2, TM // 2, 128), BF16),
            vmem((7, F // 256, TM // 2, 128), BF16),
            vmem((G, WIN + PAD, 128), F32), vmem((G, WIN + PAD, 128), F32),
            vmem((G, WIN + 2 * PAD, 128), BF16), vmem((G, WIN + 2 * PAD, 128), BF16),
            vmem((G, 64, 128), jnp.uint32), vmem((8, 128), jnp.uint32),
            pltpu.SemaphoreType.DMA((13,)), pltpu.SemaphoreType.DMA((S // TM + 1,)),
        ],
        compiler_params=pltpu.CompilerParams(
            vmem_limit_bytes=100 * 2**20, flags={"XLA_TPU_EVENLY_DISTRIBUTE_CRITICAL_NODES": True}),
    )(A_x.reshape(S, D), A_wqkv, A_wo, B_w_gate, B_w_up, B_w_down)
    return out.reshape(B, S, D)
```
